```python
import jax
import jax.numpy as jnp

def _softmax(x, axis=-1):
    return jax.nn.softmax(x, axis=axis)
def _gelu(x):
    return jax.nn.gelu(x, approximate=True)
def _silu(x):
    return jax.nn.silu(x)
def _sigmoid(x):
    return jax.nn.sigmoid(x)
def _layernorm(x, axis=-1, eps=1e-5):
    m = jnp.mean(x, axis=axis, keepdims=True)
    v = jnp.var(x, axis=axis, keepdims=True)
    return (x - m) / jnp.sqrt(v + eps)
def _scatter_add(tgt, idx, src, axis=0):
    return tgt.at[idx].add(src)
def _segment_sum(src, seg, n):
    return jax.ops.segment_sum(src, seg, n)
class _Rng:
    def __init__(self, key):
        self._k = key
    def _next(self):
        self._k, sub = jax.random.split(self._k)
        return sub
    def normal(self, shape):
        return jax.random.normal(self._next(), shape, dtype=jnp.bfloat16)
    def randint(self, lo, hi, shape):
        return jax.random.randint(self._next(), shape, lo, hi, dtype=jnp.int32)
    def uniform(self, shape, lo=0.0, hi=1.0):
        return jax.random.uniform(self._next(), shape, jnp.bfloat16, lo, hi)
    def permutation(self, n):
        return jax.random.permutation(self._next(), n)


kernel_name = 'interleave_layers__sliding_local_dilated__dense_activation_squared_relu__prompt'

def setup_inputs():
    _rng = _Rng(jax.random.key(int.from_bytes(__import__("os").urandom(4), "little")))
    _w = (lambda a: (lambda t: t.astype(jnp.bfloat16) if jnp.issubdtype(t.dtype, jnp.floating) else t)(jnp.asarray(a)))
    def _A_setup():
        B, S, D = 1, 2048, 1024
        return {
            "x": _w((lambda *s: _rng.normal(s) * 0.05)(B, S, D)),
            "wqkv": _w((lambda *s: _rng.normal(s) * 0.05)(D, 3 * D)),
            "wo": _w((lambda *s: _rng.normal(s) * 0.05)(D, D)),
        }
    _A_in = _A_setup()

    def _B_setup():
        B, S, D, F = 1, 2048, 1024, 3584
        return {
            "x": _w((lambda *s: _rng.normal(s) * 0.05)(B, S, D)),
            "w1": _w((lambda *s: _rng.normal(s) * 0.05)(D, F)),
            "b1": _w((lambda *s: _rng.normal(s) * 0.05)(F)),
            "w2": _w((lambda *s: _rng.normal(s) * 0.05)(F, D)),
            "b2": _w((lambda *s: _rng.normal(s) * 0.05)(D)),
        }
    _B_in = _B_setup()

    return {
        "A_x": _A_in["x"],
        "A_wqkv": _A_in["wqkv"],
        "A_wo": _A_in["wo"],
        "B_x": _B_in["x"],
        "B_w1": _B_in["w1"],
        "B_b1": _B_in["b1"],
        "B_w2": _B_in["w2"],
        "B_b2": _B_in["b2"],
    }

def reference(A_x, A_wqkv, A_wo, B_x, B_w1, B_b1, B_w2, B_b2):
    def _A_ref(x, wqkv, wo):
        B, S, D = x.shape
        H = 32; Dh = D // H
        W, dil = 8, 2
        qkv = (lambda x, *d: x.transpose(*d))((x @ wqkv).reshape(B, S, 3, H, Dh), 2, 0, 3, 1, 4)
        q, k, v = qkv[0], qkv[1], qkv[2]
        scale = Dh ** -0.5
        pos = jnp.arange(S)
        off = jnp.arange(W) * dil
        idx = pos[:, None] - off[None, :]
        mask = idx >= 0
        idx_c = jnp.where(mask, idx, 0).reshape(-1)
        kg = k[:, :, idx_c, :].reshape(B, H, S, W, Dh)
        vg = v[:, :, idx_c, :].reshape(B, H, S, W, Dh)
        logits = jnp.einsum("bhsd,bhswd->bhsw", q, kg) * scale
        logits = jnp.where(mask[None, None, :, :], logits, -1e9)
        attn = _softmax(logits, axis=-1)
        o = jnp.einsum("bhsw,bhswd->bhsd", attn, vg)
        return (lambda x, *d: x.transpose(*d))(o, 0, 2, 1, 3).reshape(B, S, D) @ wo

    def _B_ref(x, w1, b1, w2, b2):
        h = jnp.einsum("bsd,df->bsf", x, w1) + b1
        zero = jnp.zeros_like(h)
        r = jnp.where(h > zero, h, zero)
        h = r * r
        out = jnp.einsum("bsf,fd->bsd", h, w2) + b2
        return out

    x = A_x
    x = x + _A_ref(_layernorm(x, axis=-1), A_wqkv, A_wo)
    x = x + _B_ref(_layernorm(x, axis=-1), B_w1, B_b1, B_w2, B_b2)
    x = x + _A_ref(_layernorm(x, axis=-1), A_wqkv, A_wo)
    x = x + _B_ref(_layernorm(x, axis=-1), B_w1, B_b1, B_w2, B_b2)
    return x
```

```python
import functools
import jax
import jax.numpy as jnp
import jax.experimental.pallas as pl
import jax.experimental.pallas.tpu as pltpu

S, D, F = 2048, 1024, 3584
H, DH, W, DIL = 32, 32, 8, 2
NC = D // 128
HALO = 16
EPS = 1e-5
NEG = -1e9
SCALE = DH ** -0.5
f32, bf16, i32 = jnp.float32, jnp.bfloat16, jnp.int32


def _dot(a, b):
    return jnp.dot(a, b, preferred_element_type=f32)


def _ln(x):
    m = jnp.mean(x, axis=-1, keepdims=True)
    c = x - m
    v = jnp.mean(c * c, axis=-1, keepdims=True)
    return c * jax.lax.rsqrt(v + EPS)


def _drain(gen):
    for _ in gen:
        pass


def _paced(gen, n_steps, tokens, gate):
    for s in range(n_steps):
        gate(tokens[s * len(tokens) // n_steps]())
        if next(gen, None) is None:
            return


def _vregs(x):
    return [functools.partial(lambda r, c: x[r:r + 8, c:c + 128], r, c)
            for c in range(0, x.shape[1], 128) for r in range(0, x.shape[0], 8)]


def make(T=256, FC=512, AR=16, QC=1024, PR=64, LR=16, CG=1, NT_=0, LNB=3, L2B=12):
    NT = S // T
    NI = 2 * NT

    def permute_cols(raw, dst, part, r0):
        shape = (PR // 2, 128)
        lane = jax.lax.broadcasted_iota(i32, shape, 1)
        cols = [pl.ds(pl.multiple_of(part * D + c * 128, 128), 128) for c in range(NC)]
        b = [pltpu.bitcast(raw[pl.ds(r0, PR), cols[c]], i32) for c in range(NC)]
        b = [x if c == 0 else pltpu.roll(x, 4 * c, 1) for c, x in enumerate(b)]
        b = [b[-c % NC] for c in range(NC)]
        for bit in range(3):
            m = (lane & (4 << bit)) != 0
            b = [jnp.where(m, b[(c - (1 << bit)) % NC], b[c]) for c in range(NC)]
        for c in range(NC):
            src = (((lane & 3) << 5) + (lane & 28) + 4 * c + (lane >> 5)) & 127
            y = jnp.take_along_axis(b[c], src, axis=1)
            dst[pl.ds(r0, PR), cols[c]] = pltpu.bitcast(y, bf16)

    def kernel(x0_ref, xn_ref, wqkv_hbm, wo_hbm, w1_hbm, b1_ref, w2_hbm, b2_ref, o_ref,
               wqkv_raw, wo_raw, w1, w2, wqkv, wo, wo_f, bias1, bias2,
               xs, ln1, ln2, qkv_s, kt_s, vt_s, o_s, zero_s, sems):
        u = pl.program_id(0)

        def qkv_copy(j):
            cols = pl.ds(pl.multiple_of(j * D, D), D)
            return pltpu.make_async_copy(wqkv_hbm.at[:, cols], wqkv_raw.at[:, cols], sems.at[j])
        cp_wo = pltpu.make_async_copy(wo_hbm, wo_raw, sems.at[3])
        cp_w1 = pltpu.make_async_copy(w1_hbm, w1, sems.at[4])
        cp_w2 = pltpu.make_async_copy(w2_hbm, w2, sems.at[5])

        def qkv_cols(n0, n):
            r = _dot(ln1[...], wqkv[:, pl.ds(n0, n)])
            for cc in range(n // 128):
                qkv_s[n0 // 128 + cc, HALO:HALO + T, :] = r[:, cc * 128:(cc + 1) * 128]
            return r

        def halo(tile, pair):
            for c in range(NC):
                qkv_s[NC + c, 0:HALO, :] = kt_s[pair, c]
                v0 = jnp.broadcast_to(qkv_s[2 * NC + c, HALO:HALO + 1, :], (HALO, 128))
                qkv_s[2 * NC + c, 0:HALO, :] = jnp.where(tile == 0, v0, vt_s[pair, c])
                kt_s[pair, c] = qkv_s[NC + c, T:T + HALO, :]
                vt_s[pair, c] = qkv_s[2 * NC + c, T:T + HALO, :]

        def attn_rows(r0, tile):
            lg = [None] * W
            for c in range(NC):
                q = qkv_s[c, pl.ds(r0 + HALO, AR), :]
                for w in range(W):
                    t = q * qkv_s[NC + c, pl.ds(r0 + (HALO - DIL * w), AR), :]
                    lg[w] = t if c == 0 else lg[w] + t
                if c % CG == CG - 1 and c < NC - 1:
                    yield True
            for w in range(W):
                t = lg[w]
                t = t + pltpu.roll(t, 64, 1)
                t = t + pltpu.roll(t, 32, 1)
                t = t * SCALE
                if tile is not None:
                    pos = tile * T + r0 + jax.lax.broadcasted_iota(i32, (AR, 128), 0)
                    t = jnp.where(pos >= DIL * w, t, NEG)
                lg[w] = t
            m = functools.reduce(jnp.maximum, lg)
            e = [jnp.exp(t - m) for t in lg]
            inv = 1.0 / functools.reduce(jnp.add, e)
            yield True
            for c in range(NC):
                acc = None
                for w in range(W):
                    t = e[w] * qkv_s[2 * NC + c, pl.ds(r0 + (HALO - DIL * w), AR), :]
                    acc = t if acc is None else acc + t
                o_s[pl.ds(r0, AR), c * 128:(c + 1) * 128] = (acc * inv).astype(bf16)
                if c % CG == CG - 1:
                    yield True

        def attn(tile):
            for r0 in range(0, T, AR):
                yield from attn_rows(r0, tile if r0 < HALO else None)

        def gate(buf, dt):
            def g(tok):
                z = pl.multiple_of(zero_s[0], 8)
                idx = (0,) * (len(buf.shape) - 2) + (pl.ds(z, 8), slice(0, 128))
                buf[idx] = tok
            return g

        def ffn_up(n0):
            return _dot(ln2[...], w1[:, pl.ds(n0, FC)]) + bias1[0:1, pl.ds(n0, FC)]

        def ffn_down(n0, t, acc):
            t = jnp.where(t > 0, t, 0.0)
            return acc + _dot((t * t).astype(bf16), w2[pl.ds(n0, FC), :])

        @pl.when(u == 0)
        def _prologue():
            for cp in (qkv_copy(0), qkv_copy(1), qkv_copy(2), cp_wo, cp_w1, cp_w2):
                cp.start()
            zero_s[0] = HALO + T
            xs[1] = jnp.zeros(xs.shape[1:], f32)

            @pl.loop(0, T // 32)
            def _(j):
                rows = pl.ds(pl.multiple_of(j * 32, 32), 32)
                x = x0_ref[rows, :].astype(f32)
                xs[0, rows, :] = x
                ln1[rows, :] = _ln(x).astype(bf16)
            kt_s[...] = jnp.zeros(kt_s.shape, f32)
            vt_s[...] = jnp.zeros(vt_s.shape, f32)
            bias1[...] = jnp.broadcast_to(b1_ref[...].astype(f32).reshape(1, F), (8, F))
            bias2[...] = jnp.broadcast_to(b2_ref[...].astype(f32).reshape(1, D), (8, D))

            @pl.loop(0, 3)
            def _(part):
                qkv_copy(part).wait()

                @pl.loop(0, D // PR)
                def _(j):
                    permute_cols(wqkv_raw, wqkv, part, pl.multiple_of(j * PR, PR))

                @pl.loop(0, 2)
                def _(j):
                    qkv_cols(pl.multiple_of(part * D + j * 512, 512), 512)
            halo(0, 0)

            @pl.loop(0, T // AR)
            def _(j):
                _drain(attn_rows(pl.multiple_of(j * AR, AR), 0))
            cp_wo.wait()

            @pl.loop(0, NC)
            def _(c):
                cols = pl.ds(pl.multiple_of(c * 128, 128), 128)
                wo_f[...] = wo_raw[:, cols].astype(f32)
                for j in range(DH):
                    wo[j * H:(j + 1) * H, cols] = wo_f[pl.ds(j, H, stride=DH), :].astype(bf16)
            cp_w1.wait()
            cp_w2.wait()

        @pl.when(jnp.logical_and(u > 0, u < NI))
        def _main():
            cur = u & 1
            prv = 1 - cur
            pair = (u >> 1) & 1
            tile = ((u >> 2) << 1) + (u & 1)

            def ln1_steps():
                for r in range(0, T, LR):
                    x = jnp.where(pair == 0, xn_ref[r:r + LR, :].astype(f32), xs[cur, r:r + LR, :])
                    xs[cur, r:r + LR, :] = x
                    ln1[r:r + LR, :] = _ln(x).astype(bf16)
                    yield True

            def ln2_steps():
                for r in range(0, T, LR):
                    ln2[r:r + LR, :] = _ln(xs[prv, r:r + LR, :]).astype(bf16)
                    yield True

            x = xs[prv, 0:T, :] + _dot(o_s[...], wo[...])
            g = ln1_steps()
            _paced(g, T // LR, _vregs(x[:, :LNB * 128]), gate(xs, f32))
            _drain(g)
            xs[prv, 0:T, :] = x
            g = ln2_steps()
            toks = []
            for n0 in range(0, 3 * D, QC):
                toks += _vregs(qkv_cols(n0, QC))
            _paced(g, T // LR, toks[:L2B * 32], gate(xs, f32))
            _drain(g)
            halo(tile, pair)
            acc = xs[prv, 0:T, :] + bias2[0:1, :]
            nch = F // FC
            g = attn(tile)
            total = (T // AR) * (2 * NC // CG)
            ga = gate(qkv_s, f32)
            for j in range(nch):
                n = (j + 1) * total // nch - j * total // nch
                n1 = n * NT_ // 3
                t = ffn_up(j * FC)
                _paced(g, n1, _vregs(t), ga)
                acc = ffn_down(j * FC, t, acc)
                _paced(g, n - n1, _vregs(acc) if j < nch - 1 else _vregs(acc[:, :512]), ga)
            _drain(g)
            xs[prv, 0:T, :] = acc
            o_ref[...] = acc.astype(o_ref.dtype)

        @pl.when(u == NI)
        def _epilogue():
            @pl.loop(0, 2)
            def _(j):
                cols = pl.ds(pl.multiple_of(j * 512, 512), 512)
                xs[1, 0:T, cols] += _dot(o_s[...], wo[:, cols])

            @pl.loop(0, T // 32)
            def _(j):
                rows = pl.ds(pl.multiple_of(j * 32, 32), 32)
                x = xs[1, rows, :]
                ln2[rows, :] = _ln(x).astype(bf16)
                xs[1, rows, :] = x + bias2[0:1, :]

            @pl.loop(0, F // FC)
            def _(j):
                n0 = pl.multiple_of(j * FC, FC)
                xs[1, 0:T, :] = ffn_down(n0, ffn_up(n0), xs[1, 0:T, :])
            o_ref[...] = xs[1, 0:T, :].astype(o_ref.dtype)

    def in_idx(u):
        return jnp.minimum(((u >> 2) << 1) + jnp.minimum(u & 3, 2), NT - 1), 0

    def out_idx(u):
        j = jnp.maximum(u - 1, 0)
        return ((j >> 2) << 1) + ((j & 3) == 3).astype(i32), 0

    def fn(A_x, A_wqkv, A_wo, B_x, B_w1, B_b1, B_w2, B_b2):
        del B_x
        x = A_x.reshape(S, D)
        hbm = pl.BlockSpec(memory_space=pl.ANY)
        vm = pltpu.VMEM
        out = pl.pallas_call(
            kernel,
            grid=(NI + 1,),
            in_specs=[
                pl.BlockSpec((T, D), lambda u: (0, 0)),
                pl.BlockSpec((T, D), in_idx),
                hbm, hbm, hbm,
                pl.BlockSpec((F,), lambda u: (0,)),
                hbm,
                pl.BlockSpec((D,), lambda u: (0,)),
            ],
            out_specs=pl.BlockSpec((T, D), out_idx),
            out_shape=jax.ShapeDtypeStruct((S, D), A_x.dtype),
            scratch_shapes=[
                vm((D, 3 * D), bf16), vm((D, D), bf16), vm((D, F), bf16), vm((F, D), bf16),
                vm((D, 3 * D), bf16), vm((D, D), bf16), vm((D, 128), f32), vm((8, F), f32), vm((8, D), f32),
                vm((2, T + HALO + 8, D), f32), vm((T, D), bf16), vm((T, D), bf16),
                vm((3 * NC, HALO + T + 8, 128), f32),
                vm((2, NC, HALO, 128), f32), vm((2, NC, HALO, 128), f32),
                vm((T, D), bf16), pltpu.SMEM((1,), i32),
                pltpu.SemaphoreType.DMA((6,)),
            ],
            compiler_params=pltpu.CompilerParams(
                dimension_semantics=("arbitrary",), vmem_limit_bytes=110 * 2**20),
        )(x, x, A_wqkv, A_wo, B_w1, B_b1, B_w2, B_b2)
        return out.reshape(A_x.shape)
    return fn


_impl = make(NT_=1)


@jax.jit
def pallas_interleave_layers__sliding_local_dilated__dense_activation_squared_relu__prompt_kernel(A_x, A_wqkv, A_wo, B_x, B_w1, B_b1, B_w2, B_b2):
    return _impl(A_x, A_wqkv, A_wo, B_x, B_w1, B_b1, B_w2, B_b2)
```

```python
import functools
import jax
import jax.numpy as jnp
import jax.experimental.pallas as pl
import jax.experimental.pallas.tpu as pltpu

S, D, F = 2048, 1024, 3584
H, DH, W, DIL = 32, 32, 8, 2
NC = D // 128
HALO = 16
EPS = 1e-5
NEG = -1e9
SCALE = DH ** -0.5
LOG2E = 1.4426950408889634
f32, bf16, i32 = jnp.float32, jnp.bfloat16, jnp.int32


def _when(cond, name):
    def deco(f):
        with jax.named_scope(name):
            pl.when(cond)(f)
    return deco


def _loop(n, name):
    def deco(f):
        with jax.named_scope(name):
            pl.loop(0, n)(f)
    return deco


def _dot(a, b):
    return jnp.dot(a, b, preferred_element_type=f32)


def _pack(x):
    return pltpu.bitcast(x.astype(bf16), i32)


def _unpack(x):
    return pltpu.bitcast(x, bf16)


def _ln(x):
    m = jnp.mean(x, axis=-1, keepdims=True)
    c = x - m
    v = jnp.mean(c * c, axis=-1, keepdims=True)
    return c * jax.lax.rsqrt(v + EPS)


def _drain(gen):
    for _ in gen:
        pass


def _paced(gen, n_steps, tokens, gate):
    for s in range(n_steps):
        if next(gen):
            gate(tokens[s * len(tokens) // n_steps]())


def _steps(*gens):
    for g in gens:
        yield from g


def _vregs(x):
    return [functools.partial(lambda r, c: x[r:r + 8, c:c + 128], r, c)
            for c in range(0, x.shape[1], 128) for r in range(0, x.shape[0], 8)]


def _ds(start, size):
    if isinstance(start, int):
        return pl.ds(start, size)
    return pl.ds(pl.multiple_of(start, size), size)


def make(T=256, FC=512, AR=16, PR=32, LR=16, LC=64, UP3=2, L2B=12, ACH=6, PJ=2, TA=200, TB=250, PAD=0, IDLE=3, XP=1, WC=256, L0=10, L1=13, TQ=100, FA=3, FB=128, FC_=64, FD=200):
    NT = S // T
    NI = 2 * NT
    NCH = F // FC
    SLOTS = 2 * NC + IDLE
    KH = D // 2

    def permute_cols(raw, r0, c0, dsts, nr):
        lane = jax.lax.broadcasted_iota(i32, (nr // 2, 128), 1)
        b = [_pack(raw[_ds(r0, nr), _ds(c0 + c * 128, 128)]) for c in range(NC)]
        b = [x if c == 0 else pltpu.roll(x, 4 * c, 1) for c, x in enumerate(b)]
        b = [b[-c % NC] for c in range(NC)]
        for bit in range(3):
            m = (lane & (4 << bit)) != 0
            b = [jnp.where(m, b[(c - (1 << bit)) % NC], b[c]) for c in range(NC)]
        for c in range(NC):
            y = b[c] if c == 0 else pltpu.roll(b[c], 128 - 4 * c, 1)
            for dst, rd, cd in dsts:
                dst[_ds(rd, nr // 2), _ds(cd + c * 128, 128)] = y

    def permute_rows(raw, dst, cols, width):
        sub = jax.lax.broadcasted_iota(i32, (8, width), 0)
        for j in range(8):
            v = [_pack(raw[c * 128 + j * 16:c * 128 + (j + 1) * 16, cols]) for c in range(NC)]
            for bit in range(2):
                dl = 2 << bit
                m = (sub & dl) != 0
                for c in range(NC):
                    if not c & (1 << bit):
                        x, y = v[c], v[c | (1 << bit)]
                        v[c] = jnp.where(m, pltpu.roll(y, dl, 0), x)
                        v[c | (1 << bit)] = jnp.where(m, y, pltpu.roll(x, 8 - dl, 0))
            for c in range(NC):
                r = (((j & 1) << 2) | (c & 3)) * 64 + ((j >> 1) * 2 + (c >> 2)) * 8
                dst[r:r + 8, cols] = v[c]

    def kernel(x_hbm, wqkv_hbm, wo_hbm, w1_hbm, b1_ref, w2_hbm, b2_ref, o_ref,
               x_in, wqkv_raw, wo_raw, w1, w2, wqkv, w_a, w_b, wo, bias1, bias2,
               xs, x2, ln1, ln2, qkv_s, qkv_0, o_s, spare, sems):
        u = pl.program_id(0)

        def qkv_copy(j):
            blk = (_ds((j & 1) * KH, KH), _ds((j >> 1) * D, D))
            return pltpu.make_async_copy(wqkv_hbm.at[blk], wqkv_raw.at[blk], sems.at[j])

        def w1_copy(j):
            cols = _ds(j * FC, FC)
            return pltpu.make_async_copy(w1_hbm.at[:, cols], w1.at[:, cols], sems.at[10 + j])

        def w2_copy(j):
            rows = _ds(j * FC, FC)
            return pltpu.make_async_copy(w2_hbm.at[rows, :], w2.at[rows, :], sems.at[10 + NCH + j])
        cp_wo = pltpu.make_async_copy(wo_hbm.at[:, :], wo_raw.at[0:D, :], sems.at[6])
        cp_x = [pltpu.make_async_copy(x_hbm.at[a * T:b * T, :], x_in.at[a * T:b * T, :], sems.at[7 + j])
                for j, (a, b) in enumerate(((0, 1), (1, 3), (3, NT)))]

        def gate(buf):
            def g(tok):
                if buf.dtype == bf16:
                    z = pl.multiple_of(spare[1], 16)
                    buf[pl.ds(z, 16), 0:128] = jnp.concatenate([tok, tok], axis=0).astype(bf16)
                else:
                    z = pl.multiple_of(spare[2 if buf.dtype == i32 else 0], 8)
                    buf[(0,) * (len(buf.shape) - 2) + (pl.ds(z, 8), slice(0, 128))] = (
                        tok if buf.dtype == f32 else pltpu.bitcast(tok, i32))
            return g

        def first_tile_halo(buf, tile):
            for c in range(2 * NC, 3 * NC):
                v0 = jnp.broadcast_to(buf[c, HALO:HALO + 1, :], (HALO, 128))
                buf[c, 0:HALO, :] = jnp.where(tile == 0, v0, buf[c, 0:HALO, :])

        def attn_rows(buf, r0, pos0):
            def rows(c, w):
                return buf[c, pl.ds(r0 + (HALO - DIL * w), AR), :]
            lg = [None] * W
            for c in range(NC):
                yield True
                q = rows(c, 0)
                for w in range(W):
                    t = q * rows(NC + c, w)
                    lg[w] = t if c == 0 else lg[w] + t
            if XP:
                t = jnp.concatenate(lg, axis=0)
                lane = jax.lax.broadcasted_iota(i32, t.shape, 1)
                t = t + jnp.take_along_axis(t, lane ^ 1, axis=1)
                t = t + jnp.take_along_axis(t, lane ^ 2, axis=1)
                lg = [t[w * AR:(w + 1) * AR] for w in range(W)]
            else:
                lane = jax.lax.broadcasted_iota(i32, (AR, 128), 1)
                for w in range(W):
                    t = lg[w]
                    t = t + jnp.where((lane & 1) != 0, pltpu.roll(t, 1, 1), pltpu.roll(t, 127, 1))
                    lg[w] = t + jnp.where((lane & 2) != 0, pltpu.roll(t, 2, 1), pltpu.roll(t, 126, 1))
            if pos0 is not None:
                pos = pos0 + jax.lax.broadcasted_iota(i32, (AR, 128), 0)
                lg = [jnp.where(pos >= DIL * w, lg[w], NEG / SCALE) for w in range(W)]
            m = functools.reduce(jnp.maximum, lg)
            e = [jnp.exp2((t - m) * (SCALE * LOG2E)) for t in lg]
            inv = 1.0 / functools.reduce(jnp.add, e)
            for _ in range(IDLE):
                yield False
            for c in range(NC):
                yield True
                acc = None
                for w in range(W):
                    t = e[w] * rows(2 * NC + c, w)
                    acc = t if acc is None else acc + t
                o_s[_ds(r0 // 2, AR // 2), c * 128:(c + 1) * 128] = _pack(acc * inv)

        def ln1_rows(r, nr, item):
            yield True
            tile = item & (NT - 1)
            x = jnp.where(item < NT, x_in[_ds(tile * T + r, nr), :].astype(f32), xs[tile, _ds(r, nr), :])
            xs[tile, _ds(r, nr), :] = x
            ln1[_ds(r // 2, nr // 2), :] = _pack(_ln(x))

        def ffn_up(cols):
            return _dot(_unpack(ln2[0:T // 2, :]), w1[:, cols]) + bias1[0:1, cols]

        def ffn_down(cols, t, acc):
            t = jnp.maximum(t, 0.0)
            return acc + _dot((t * t).astype(bf16), w2[cols, :])

        def share(j, n_iter, n):
            per = -(-n // n_iter)
            return [pl.multiple_of(jnp.minimum(j * per + i, n - 1) * (T // n), T // n) for i in range(per)]

        edge = jnp.logical_or(u == 0, u == NT * 2 - 1)

        @_when(jnp.logical_not(edge), "steady")
        def _steady():
            done, cur = u & (NT - 1), (u + 1) & (NT - 1)

            def ln2_steps():
                for r in range(0, T, LR):
                    yield True
                    ln2[r // 2:(r + LR) // 2, :] = _pack(_ln(x2[r:r + LR, :]))

            for c in range(NC, 3 * NC):
                qkv_s[c, 0:HALO, :] = qkv_s[c, T:T + HALO, :]
            x2[0:T, :] = xs[done, 0:T, :] + _dot(_unpack(o_s[...]), _unpack(wo[...]))
            toks = []
            a = _unpack(ln1[...])
            for n0 in range(0, 3 * D, D):
                r = _dot(a, _unpack(wqkv[:, n0:n0 + D]))
                for c in range(NC):
                    qkv_s[n0 // 128 + c, HALO:HALO + T, :] = r[:, c * 128:(c + 1) * 128]
                toks += _vregs(r)
            g = ln2_steps()
            _paced(g, T // LR, toks[:L2B * 32], gate(x2))
            _drain(g)
            first_tile_halo(qkv_s, cur)
            acc = x2[0:T, :] + bias2[0:1, :]
            ga = _steps(*(attn_rows(qkv_s, r0, cur * T + r0 if r0 < HALO else None) for r0 in range(0, T, AR)))
            gl = _steps(*(ln1_rows(r, LR, u + 2) for r in range(0, T, LR)))
            total = (T // AR) * SLOTS
            def quota(n, h0, h1, h):
                return (h - h0 + 1) * n // (h1 - h0) - (h - h0) * n // (h1 - h0) if h0 <= h < h1 else 0
            for j in range(NCH):
                cols = pl.ds(j * FC, FC)
                t = ffn_up(cols)
                n = quota(total, 0, ACH, j)
                n1 = n * UP3 // 6
                _paced(gl, quota(T // LR, L0, L1, 2 * j), _vregs(t), gate(xs))
                _paced(ga, n1, _vregs(t), gate(qkv_s))
                acc = ffn_down(cols, t, acc)
                _paced(gl, quota(T // LR, L0, L1, 2 * j + 1), _vregs(acc), gate(xs))
                _paced(ga, n - n1, _vregs(acc), gate(qkv_s))
            _drain(ga)
            _drain(gl)
            xs[done, 0:T, :] = acc
            o_ref[...] = acc.astype(o_ref.dtype)

        @pl.when(u == 0)
        def _start():
            for cp in (cp_x[0], *(qkv_copy(j) for j in range(6)), cp_x[1], cp_wo):
                cp.start()
            for j in range(NCH):
                w1_copy(j).start()
                w2_copy(j).start()
            cp_x[2].start()
            spare[0] = HALO + T
            spare[1] = D
            spare[2] = KH // 2
            qkv_0[NC:2 * NC, 0:HALO, :] = jnp.zeros((NC, HALO, 128), f32)
            bias1[...] = jnp.broadcast_to(b1_ref[...].astype(f32).reshape(1, F), (8, F))
            bias2[...] = jnp.broadcast_to(b2_ref[...].astype(f32).reshape(1, D), (8, D))
            cp_x[0].wait()

            @_loop(T // LC, "ln_first")
            def _(i):
                x = x_in[_ds(i * LC, LC), :].astype(f32)
                xs[0, _ds(i * LC, LC), :] = x
                ln2[_ds(i * (LC // 2), LC // 2), :] = _pack(_ln(x))
            qkv_copy(0).wait()

            @_loop(2, "perm")
            def _(j):
                permute_cols(wqkv_raw, j * (KH // 2), 0, [(w_a, j * (KH // 4), 0), (wqkv, j * (KH // 4), 0)], KH // 2)

            @_loop(3, "qkv0")
            def _(p):
                for kh, (src, dst) in enumerate(((w_a, w_b), (w_b, w_a))):
                    nxt = jnp.minimum(2 * p + kh + 1, 5)

                    @pl.when(2 * p + kh < 5)
                    def _():
                        qkv_copy(nxt).wait()
                    r = _dot(_unpack(ln2[0:T // 2, kh * KH:(kh + 1) * KH]), _unpack(src[...]))
                    for c in range(NC):
                        blk = (p * NC + c, slice(HALO, HALO + T), slice(None))
                        part = r[:, c * 128:(c + 1) * 128]
                        qkv_0[blk] = qkv_0[blk] + part if kh else part
                    toks = _vregs(r)
                    for s in range(KH // PR):
                        gate(wqkv_raw)(toks[s * TA // (KH // PR)]())
                        r0, c0 = (1 - kh) * KH + s * PR, (nxt >> 1) * D
                        permute_cols(wqkv_raw, r0, c0, [(dst, s * PR // 2, 0), (wqkv, r0 // 2, c0)], PR)
            cp_x[1].wait()
            cp_wo.wait()

            @_loop(T // LC, "ln_second")
            def _(i):
                _drain(ln1_rows(i * LC, LC, 1))
            first_tile_halo(qkv_0, 0)
            for c in range(NC, 3 * NC):
                qkv_s[c, 0:HALO, :] = qkv_0[c, T:T + HALO, :]

            @_loop(6, "qkv1")
            def _(j):
                r = _dot(_unpack(ln1[...]), _unpack(wqkv[:, _ds(j * 512, 512)]))
                for c in range(4):
                    qkv_s[j * 4 + c, HALO:HALO + T, :] = r[:, c * 128:(c + 1) * 128]
                chunks = share(j, 6, T // AR)
                ga = _steps(*(attn_rows(qkv_0, r0, r0) for r0 in chunks))
                _paced(ga, len(chunks) * SLOTS, _vregs(r)[:TQ], gate(qkv_0))
                _drain(ga)

            @_loop(D // WC, "perm_wo")
            def _(c):
                permute_rows(wo_raw, wo, _ds(c * WC, WC), WC)

        @_when(edge, "edge")
        def _edge():
            done = u & (NT - 1)

            @_loop(PJ, "proj")
            def _(j):
                cols = _ds(j * (D // PJ), D // PJ)
                x2[0:T, cols] = xs[done, 0:T, cols] + _dot(_unpack(o_s[...]), _unpack(wo[:, cols]))

            @_loop(T // LC, "ln2")
            def _(j):
                x = x2[_ds(j * LC, LC), :]
                ln2[_ds(j * (LC // 2), LC // 2), :] = _pack(_ln(x))
                x2[_ds(j * LC, LC), :] = x + bias2[0:1, :]

            @_loop(NCH, "ffn")
            def _(j):
                @pl.when(u == 0)
                def _():
                    w1_copy(j).wait()
                    w2_copy(j).wait()
                cols = _ds(j * FC, FC)
                t = ffn_up(cols)
                chunks = share(j, NCH, T // AR)
                pos = ((u + 1) & (NT - 1)) * T
                ga = _steps(*(attn_rows(qkv_s, r0, pos + r0) for r0 in chunks))
                n = len(chunks) * SLOTS
                _paced(ga, n * FA // 6, _vregs(t), gate(qkv_s))
                acc = ffn_down(cols, t, x2[0:T, :])
                x2[0:T, :] = acc
                _paced(ga, n - n * FA // 6, _vregs(acc)[:FB], gate(qkv_s))
                _drain(ga)
                chunks = share(j, NCH, T // LR)
                gl = _steps(*(ln1_rows(r, LR, u + 2) for r in chunks))
                _paced(gl, len(chunks), _vregs(acc)[FC_:FD], gate(xs))
                _drain(gl)
            xs[done, 0:T, :] = x2[0:T, :]
            o_ref[...] = x2[0:T, :].astype(o_ref.dtype)

            @pl.when(u == 0)
            def _():
                cp_x[2].wait()
        if PAD:
            @pl.when(u == spare[0])
            def _():
                for i in range(PAD):
                    x2[0:T, :] = _dot(_unpack(ln1[...]), w1[:, i * 512:i * 512 + 1024])

    def fn(A_x, A_wqkv, A_wo, B_x, B_w1, B_b1, B_w2, B_b2):
        del B_x
        x = A_x.reshape(S, D)
        hbm = pl.BlockSpec(memory_space=pl.ANY)
        vm = pltpu.VMEM
        out = pl.pallas_call(
            kernel,
            grid=(NI,),
            in_specs=[
                hbm, hbm, hbm, hbm,
                pl.BlockSpec((F,), lambda u: (0,)),
                hbm,
                pl.BlockSpec((D,), lambda u: (0,)),
            ],
            out_specs=pl.BlockSpec((T, D), lambda u: (jnp.maximum(u - NT, 0), 0)),
            out_shape=jax.ShapeDtypeStruct((S, D), A_x.dtype),
            scratch_shapes=[
                vm((S, D), bf16), vm((D + 16, 3 * D), bf16), vm((D, D), bf16), vm((D, F), bf16), vm((F, D), bf16),
                vm((KH, 3 * D), i32), vm((KH // 2, D), i32), vm((KH // 2, D), i32), vm((KH, D), i32),
                vm((8, F), f32), vm((8, D), f32),
                vm((NT, T + HALO + 8, D), f32), vm((T + HALO + 8, D), f32),
                vm((T // 2, D), i32), vm((T // 2, D), i32),
                vm((3 * NC, HALO + T + 8, 128), f32), vm((3 * NC, HALO + T + 8, 128), f32),
                vm((T // 2, D), i32), pltpu.SMEM((3,), i32),
                pltpu.SemaphoreType.DMA((10 + 2 * NCH,)),
            ],
            compiler_params=pltpu.CompilerParams(
                dimension_semantics=("arbitrary",), vmem_limit_bytes=110 * 2**20),
        )(x, A_wqkv, A_wo, B_w1, B_b1, B_w2, B_b2)
        return out.reshape(A_x.shape)
    return fn


_impl = make()


@jax.jit
def pallas_interleave_layers__sliding_local_dilated__dense_activation_squared_relu__prompt_kernel(A_x, A_wqkv, A_wo, B_x, B_w1, B_b1, B_w2, B_b2):
    return _impl(A_x, A_wqkv, A_wo, B_x, B_w1, B_b1, B_w2, B_b2)
```

```python
import functools

import jax
import jax.numpy as jnp
import jax.experimental.pallas as pl
import jax.experimental.pallas.tpu as pltpu

S, D, F = 2048, 1024, 3584
DH, W, DIL = 32, 8, 2
EPS = 1e-5
NEG = -1e9
SCALE = DH ** -0.5
LOG2E = 1.4426950408889634

T = 256
NT = S // T
NI = 2 * NT
NC = D // 128
HALO = 16
KH = D // 2
FC = 512
FE = 896
RB = 16
IDLE = 3
SLOTS = 2 * NC + IDLE
PR = 32

f32, bf16, i32 = jnp.float32, jnp.bfloat16, jnp.int32


def _dot(a, b):
    return jnp.dot(a, b, preferred_element_type=f32)


def _pack(x):
    return pltpu.bitcast(x.astype(bf16), i32)


def _unpack(x):
    return pltpu.bitcast(x, bf16)


def _ln(x):
    m = jnp.mean(x, axis=-1, keepdims=True)
    c = x - m
    v = jnp.mean(c * c, axis=-1, keepdims=True)
    return c * jax.lax.rsqrt(v + EPS)


def _ds(start, size, align=None):
    if isinstance(start, int):
        return pl.ds(start, size)
    return pl.ds(pl.multiple_of(start, align or size), size)


def _steps(*gens):
    for g in gens:
        yield from g


def _drain(gen):
    for _ in gen:
        pass


def _paced(gen, n_steps, tokens, gate):
    for s in range(n_steps):
        if next(gen):
            gate(tokens[s * len(tokens) // n_steps]())


def _vregs(x):
    return [functools.partial(lambda r, c: x[r:r + 8, c:c + 128], r, c)
            for c in range(0, x.shape[1], 128) for r in range(0, x.shape[0], 8)]


def _permute_cols(raw, r0, c0, dsts, nr):
    lane = jax.lax.broadcasted_iota(i32, (nr // 2, 128), 1)
    b = [_pack(raw[_ds(r0, nr), _ds(c0 + c * 128, 128)]) for c in range(NC)]
    b = [x if c == 0 else pltpu.roll(x, 4 * c, 1) for c, x in enumerate(b)]
    b = [b[-c % NC] for c in range(NC)]
    for bit in range(3):
        m = (lane & (4 << bit)) != 0
        b = [jnp.where(m, b[(c - (1 << bit)) % NC], b[c]) for c in range(NC)]
    for c in range(NC):
        y = b[c] if c == 0 else pltpu.roll(b[c], 128 - 4 * c, 1)
        for dst, rd, cd in dsts:
            dst[_ds(rd, nr // 2), _ds(cd + c * 128, 128)] = y


def _permute_rows(raw, dst, c0, width):
    cols = _ds(c0, width)
    sub = jax.lax.broadcasted_iota(i32, (8, width), 0)
    for j in range(8):
        v = [_pack(raw[c * 128 + j * 16:c * 128 + (j + 1) * 16, cols]) for c in range(NC)]
        for bit in range(2):
            dl = 2 << bit
            m = (sub & dl) != 0
            for c in range(NC):
                if not c & (1 << bit):
                    x, y = v[c], v[c | (1 << bit)]
                    v[c] = jnp.where(m, pltpu.roll(y, dl, 0), x)
                    v[c | (1 << bit)] = jnp.where(m, y, pltpu.roll(x, 8 - dl, 0))
        for c in range(NC):
            r = (((j & 1) << 2) | (c & 3)) * 64 + ((j >> 1) * 2 + (c >> 2)) * 8
            dst[r:r + 8, cols] = v[c]


def _kernel(x_hbm, wqkv_hbm, wo_hbm, w1_hbm, b1_hbm, w2_hbm, b2_hbm, o_hbm,
            spare, sems, x2, w2, w1, b1_raw, b2_raw, out_s, x_in, wqkv_raw, wo_raw, wqkv, w_a, w_b, wo,
            bias1, bias2, xs, x_att, ln1, ln2, qkv_s, qkv_0, o_s):
    n_edge = F // FE

    def qkv_copy(j):
        blk = (_ds((j & 1) * KH, KH), _ds((j >> 1) * D, D))
        return pltpu.make_async_copy(wqkv_hbm.at[blk], wqkv_raw.at[blk], sems.at[j])

    def x_copy(j):
        a, b = ((0, T), (T, 3 * T), (3 * T, S))[j]
        return pltpu.make_async_copy(x_hbm.at[a:b, :], x_in.at[a:b, :], sems.at[6 + j])

    def small_copy(j):
        src, dst = ((wo_hbm, wo_raw), (b1_hbm, b1_raw), (b2_hbm, b2_raw))[j]
        return pltpu.make_async_copy(src, dst, sems.at[9 + j])

    def w1_copy(j):
        cols = _ds(j * FE, FE, 128)
        return pltpu.make_async_copy(w1_hbm.at[:, cols], w1.at[:, cols], sems.at[12 + j])

    def w2_copy(j):
        rows = _ds(j * FE, FE, 128)
        return pltpu.make_async_copy(w2_hbm.at[rows, :], w2.at[rows, :], sems.at[12 + n_edge + j])

    def out_copy(t):
        return pltpu.make_async_copy(out_s.at[t], o_hbm.at[_ds(t * T, T), :], sems.at[12 + 2 * n_edge + t])

    def gate(buf):
        def store(tok):
            if buf.dtype == bf16:
                z = pl.multiple_of(spare[1], 16)
                buf[pl.ds(z, 16), 0:128] = jnp.concatenate([tok, tok], axis=0).astype(bf16)
            else:
                z = pl.multiple_of(spare[0], 8)
                buf[(0,) * (len(buf.shape) - 2) + (pl.ds(z, 8), slice(0, 128))] = tok
        return store

    def put_blocks(buf, c0, r):
        for c in range(r.shape[1] // 128):
            buf[c0 + c, HALO:HALO + T, :] = r[:, c * 128:(c + 1) * 128]

    def first_tile_halo(buf, tile):
        for c in range(2 * NC, 3 * NC):
            v0 = jnp.broadcast_to(buf[c, HALO:HALO + 1, :], (HALO, 128))
            buf[c, 0:HALO, :] = jnp.where(tile == 0, v0, buf[c, 0:HALO, :])

    def attn_rows(buf, r0, pos0):
        def rows(c, w):
            return buf[c, pl.ds(r0 + (HALO - DIL * w), RB), :]
        lg = [None] * W
        for c in range(NC):
            yield True
            q = rows(c, 0)
            for w in range(W):
                t = q * rows(NC + c, w)
                lg[w] = t if c == 0 else lg[w] + t
        t = jnp.concatenate(lg, axis=0)
        lane = jax.lax.broadcasted_iota(i32, t.shape, 1)
        t = t + jnp.take_along_axis(t, lane ^ 1, axis=1)
        t = t + jnp.take_along_axis(t, lane ^ 2, axis=1)
        lg = [t[w * RB:(w + 1) * RB] for w in range(W)]
        if pos0 is not None:
            pos = pos0 + jax.lax.broadcasted_iota(i32, (RB, 128), 0)
            lg = [jnp.where(pos >= DIL * w, lg[w], NEG / SCALE) for w in range(W)]
        m = functools.reduce(jnp.maximum, lg)
        e = [jnp.exp2((t - m) * (SCALE * LOG2E)) for t in lg]
        inv = 1.0 / functools.reduce(jnp.add, e)
        for _ in range(IDLE):
            yield False
        for c in range(NC):
            yield True
            acc = None
            for w in range(W):
                t = e[w] * rows(2 * NC + c, w)
                acc = t if acc is None else acc + t
            o_s[_ds(r0 // 2, RB // 2), c * 128:(c + 1) * 128] = _pack(acc * inv)

    def stream(item, r, nr, cols=slice(None)):
        tile = item & (NT - 1)
        return jnp.where(item < NT, x_in[_ds(tile * T + r, nr), cols].astype(f32), xs[tile, _ds(r, nr), cols])

    def ln1_rows(r, item):
        yield True
        ln1[_ds(r // 2, RB // 2), :] = _pack(_ln(stream(item, r, RB)))

    def ln2_rows(src, r):
        yield True
        ln2[r // 2:(r + RB) // 2, :] = _pack(_ln(src[r:r + RB, :]))

    def ffn_up(cols):
        return _dot(_unpack(ln2[...]), w1[:, cols]) + bias1[0:1, cols]

    def ffn_down(cols, t, acc):
        t = jnp.maximum(t, 0.0)
        return acc + _dot((t * t).astype(bf16), w2[cols, :])

    def store_out(u, y):
        out_s[jnp.maximum(u - NT, 0)] = y.astype(out_s.dtype)

    def share(j, n_iter):
        n = T // RB
        per = -(-n // n_iter)
        return [pl.multiple_of(jnp.minimum(j * per + i, n - 1) * RB, RB) for i in range(per)]

    def start():
        for cp in (x_copy(0), *(qkv_copy(j) for j in range(6)),
                   small_copy(1), small_copy(2), x_copy(1), small_copy(0)):
            cp.start()
        for j in range(n_edge):
            w1_copy(j).start()
            w2_copy(j).start()
        x_copy(2).start()
        spare[0] = HALO + T
        spare[1] = D
        qkv_0[NC:, 0:HALO, :] = jnp.zeros((2 * NC, HALO, 128), f32)

        @pl.loop(0, NT)
        def _(t):
            xs[t, 0:T, :] = jnp.zeros((T, D), f32)
        x_copy(0).wait()
        for r in range(0, T, RB):
            ln2[r // 2:(r + RB) // 2, :] = _pack(_ln(x_in[r:r + RB, :].astype(f32)))
        qkv_copy(0).wait()

        @pl.loop(0, 2)
        def _(j):
            rd = j * (KH // 4)
            _permute_cols(wqkv_raw, j * (KH // 2), 0, [(w_a, rd, 0), (wqkv, rd, 0)], KH // 2)

        @pl.loop(0, 3)
        def _(p):
            for kh, (src, dst) in enumerate(((w_a, w_b), (w_b, w_a))):
                nxt = jnp.minimum(2 * p + kh + 1, 5)

                @pl.when(2 * p + kh < 5)
                def _():
                    qkv_copy(nxt).wait()
                r = _dot(_unpack(ln2[:, kh * KH:(kh + 1) * KH]), _unpack(src[...]))
                for c in range(NC):
                    blk = (p * NC + c, slice(HALO, HALO + T), slice(None))
                    part = r[:, c * 128:(c + 1) * 128]
                    qkv_0[blk] = qkv_0[blk] + part if kh else part
                toks = _vregs(r)
                for s in range(KH // PR):
                    gate(wqkv_raw)(toks[s * 200 // (KH // PR)]())
                    r0, c0 = (1 - kh) * KH + s * PR, (nxt >> 1) * D
                    _permute_cols(wqkv_raw, r0, c0, [(dst, s * PR // 2, 0), (wqkv, r0 // 2, c0)], PR)

        for cp in (small_copy(1), small_copy(2), x_copy(1), small_copy(0)):
            cp.wait()
        bias1[...] = jnp.broadcast_to(b1_raw[...].astype(f32).reshape(1, F), (8, F))
        bias2[...] = jnp.broadcast_to(b2_raw[...].astype(f32).reshape(1, D), (8, D))
        for r in range(0, T, RB):
            ln1[r // 2:(r + RB) // 2, :] = _pack(_ln(x_in[T + r:T + r + RB, :].astype(f32)))
        first_tile_halo(qkv_0, 0)
        for c in range(NC, 3 * NC):
            qkv_s[c, 0:HALO, :] = qkv_0[c, T:T + HALO, :]

        @pl.loop(0, 3)
        def _(p):
            r = _dot(_unpack(ln1[...]), _unpack(wqkv[:, _ds(p * D, D)]))
            put_blocks(qkv_s, p * NC, r)
            pieces = share(p, 3)
            ga = _steps(*(attn_rows(qkv_0, r0, r0) for r0 in pieces))
            _paced(ga, len(pieces) * SLOTS, _vregs(r)[:210], gate(qkv_0))
            _drain(ga)

        @pl.loop(0, D // 256)
        def _(c):
            _permute_rows(wo_raw, wo, c * 256, 256)

    def steady(u):
        cur = (u + 1) & (NT - 1)
        for c in range(NC, 3 * NC):
            qkv_s[c, 0:HALO, :] = qkv_s[c, T:T + HALO, :]
        x2[0:T, :] = stream(u, 0, T) + _dot(_unpack(o_s[...]), _unpack(wo[...]))
        toks = []
        a = _unpack(ln1[...])
        for p in range(3):
            r = _dot(a, _unpack(wqkv[:, p * D:(p + 1) * D]))
            put_blocks(qkv_s, p * NC, r)
            toks += _vregs(r)
        g2 = _steps(*(ln2_rows(x2, r) for r in range(0, T, RB)))
        _paced(g2, T // RB, toks[:384], gate(x2))
        _drain(g2)
        first_tile_halo(qkv_s, cur)

        def quota(n, h0, h1, h):
            return (h - h0 + 1) * n // (h1 - h0) - (h - h0) * n // (h1 - h0) if h0 <= h < h1 else 0
        acc = x2[0:T, :] + bias2[0:1, :]
        ga = _steps(*(attn_rows(qkv_s, r0, cur * T + r0 if r0 < HALO else None) for r0 in range(0, T, RB)))
        g1 = _steps(*(ln1_rows(r, u + 2) for r in range(0, T, RB)))
        for j in range(F // FC):
            cols = pl.ds(j * FC, FC)
            n = quota((T // RB) * SLOTS, 0, 6, j)
            t = ffn_up(cols)
            _paced(g1, quota(T // RB, 11, 13, 2 * j), _vregs(t), gate(xs))
            _paced(ga, n // 3, _vregs(t), gate(qkv_s))
            acc = ffn_down(cols, t, acc)
            _paced(g1, quota(T // RB, 11, 13, 2 * j + 1), _vregs(acc), gate(xs))
            _paced(ga, n - n // 3, _vregs(acc), gate(qkv_s))
        _drain(ga)
        _drain(g1)
        xs[u & (NT - 1), 0:T, :] = acc
        store_out(u, acc)

    def edge(u):
        @pl.loop(0, 2)
        def _(j):
            cols = _ds(j * (D // 2), D // 2)
            x = stream(u, 0, T, cols) + _dot(_unpack(o_s[...]), _unpack(wo[:, cols]))
            x_att[:, cols] = x
            x2[0:T, cols] = x + bias2[0:1, cols]
        _drain(_steps(*(ln2_rows(x_att, r) for r in range(0, T, RB))))

        @pl.loop(0, n_edge)
        def _(j):
            @pl.when(u == 0)
            def _():
                w1_copy(j).wait()
                w2_copy(j).wait()
            cols = _ds(j * FE, FE, 128)
            t = ffn_up(cols)
            pieces = share(j, n_edge)
            pos = ((u + 1) & (NT - 1)) * T
            ga = _steps(*(attn_rows(qkv_s, r0, pos + r0) for r0 in pieces))
            n = len(pieces) * SLOTS
            _paced(ga, n * 2 // 3, _vregs(t), gate(qkv_s))
            acc = ffn_down(cols, t, x2[0:T, :])
            x2[0:T, :] = acc
            _paced(ga, n - n * 2 // 3, _vregs(acc)[:100], gate(qkv_s))
            _drain(ga)
            g1 = _steps(*(ln1_rows(r, u + 2) for r in pieces))
            _paced(g1, len(pieces), _vregs(acc)[100:220], gate(xs))
            _drain(g1)

        @pl.when(u == 0)
        def _():
            xs[0, 0:T, :] = x2[0:T, :]
            x_copy(2).wait()

        @pl.when(u != 0)
        def _():
            store_out(u, x2[0:T, :])

    start()

    @pl.loop(0, NI)
    def _(u):
        is_edge = jnp.logical_or(u == 0, u == NI - 1)
        pl.when(jnp.logical_not(is_edge))(lambda: steady(u))
        pl.when(is_edge)(lambda: edge(u))
        pl.when(u >= NT)(lambda: out_copy(u - NT).start())

    for t in range(NT):
        out_copy(t).wait()


@jax.jit
def pallas_interleave_layers__sliding_local_dilated__dense_activation_squared_relu__prompt_kernel(
    A_x: jax.Array,
    A_wqkv: jax.Array,
    A_wo: jax.Array,
    B_x: jax.Array,
    B_w1: jax.Array,
    B_b1: jax.Array,
    B_w2: jax.Array,
    B_b2: jax.Array,
):
    del B_x
    vm = pltpu.VMEM
    hbm = pl.BlockSpec(memory_space=pl.ANY)
    out = pl.pallas_call(
        _kernel,
        in_specs=[hbm] * 7,
        out_specs=hbm,
        out_shape=jax.ShapeDtypeStruct((S, D), A_x.dtype),
        scratch_shapes=[
            pltpu.SMEM((2,), i32),
            pltpu.SemaphoreType.DMA((12 + 2 * (F // FE) + NT,)),
            vm((T + HALO + 8, D), f32),
            vm((F, D), bf16), vm((D, F), bf16),
            vm((F,), bf16), vm((D,), bf16),
            vm((NT, T, D), A_x.dtype), vm((S, D), A_x.dtype),
            vm((D + 16, 3 * D), bf16), vm((D, D), bf16),
            vm((KH, 3 * D), i32),
            vm((KH // 2, D), i32), vm((KH // 2, D), i32),
            vm((KH, D), i32),
            vm((8, F), f32), vm((8, D), f32),
            vm((NT, T + HALO + 8, D), f32), vm((T, D), f32),
            vm((T // 2, D), i32), vm((T // 2, D), i32),
            vm((3 * NC, HALO + T + 8, 128), f32),
            vm((3 * NC, HALO + T + 8, 128), f32),
            vm((T // 2, D), i32),
        ],
        compiler_params=pltpu.CompilerParams(vmem_limit_bytes=110 * 2**20),
    )(A_x.reshape(S, D), A_wqkv, A_wo, B_w1, B_b1, B_w2, B_b2)
    return out.reshape(A_x.shape)
```

```python
import functools

import jax
import jax.numpy as jnp
import jax.experimental.pallas as pl
import jax.experimental.pallas.tpu as pltpu

S, D, F = 2048, 1024, 3584
DH, W, DIL = 32, 8, 2
EPS = 1e-5
NEG = -1e9
SCALE = DH ** -0.5
LOG2E = 1.4426950408889634

T = 256
NT = S // T
NI = 2 * NT
NC = D // 128
HALO = 16
KH = D // 2
FC = 512
FE = 896
RB = 16
IDLE = 3
SLOTS = 2 * NC + IDLE
PR = 32

f32, bf16, i32 = jnp.float32, jnp.bfloat16, jnp.int32


def _dot(a, b):
    return jnp.dot(a, b, preferred_element_type=f32)


def _pack(x):
    return pltpu.bitcast(x.astype(bf16), i32)


def _unpack(x):
    return pltpu.bitcast(x, bf16)


def _ln(x):
    m = jnp.mean(x, axis=-1, keepdims=True)
    c = x - m
    v = jnp.mean(c * c, axis=-1, keepdims=True)
    return c * jax.lax.rsqrt(v + EPS)


def _ds(start, size, align=None):
    if isinstance(start, int):
        return pl.ds(start, size)
    return pl.ds(pl.multiple_of(start, align or size), size)


def _steps(*gens):
    for g in gens:
        yield from g


def _drain(gen):
    for _ in gen:
        pass


def _paced(gen, n_steps, tokens, gate):
    for s in range(n_steps):
        if next(gen):
            gate(tokens[s * len(tokens) // n_steps]())


def _vregs(x):
    return [functools.partial(lambda r, c: x[r:r + 8, c:c + 128], r, c)
            for c in range(0, x.shape[1], 128) for r in range(0, x.shape[0], 8)]


def _permute_cols(raw, r0, c0, dsts, nr):
    lane = jax.lax.broadcasted_iota(i32, (nr // 2, 128), 1)
    b = [_pack(raw[_ds(r0, nr), _ds(c0 + c * 128, 128)]) for c in range(NC)]
    b = [x if c == 0 else pltpu.roll(x, 4 * c, 1) for c, x in enumerate(b)]
    b = [b[-c % NC] for c in range(NC)]
    for bit in range(3):
        m = (lane & (4 << bit)) != 0
        b = [jnp.where(m, b[(c - (1 << bit)) % NC], b[c]) for c in range(NC)]
    for c in range(NC):
        y = b[c] if c == 0 else pltpu.roll(b[c], 128 - 4 * c, 1)
        for dst, rd, cd in dsts:
            dst[_ds(rd, nr // 2), _ds(cd + c * 128, 128)] = y


def _permute_rows(raw, dst, c0, width):
    cols = _ds(c0, width)
    sub = jax.lax.broadcasted_iota(i32, (8, width), 0)
    for j in range(8):
        v = [_pack(raw[c * 128 + j * 16:c * 128 + (j + 1) * 16, cols]) for c in range(NC)]
        for bit in range(2):
            dl = 2 << bit
            m = (sub & dl) != 0
            for c in range(NC):
                if not c & (1 << bit):
                    x, y = v[c], v[c | (1 << bit)]
                    v[c] = jnp.where(m, pltpu.roll(y, dl, 0), x)
                    v[c | (1 << bit)] = jnp.where(m, y, pltpu.roll(x, 8 - dl, 0))
        for c in range(NC):
            r = (((j & 1) << 2) | (c & 3)) * 64 + ((j >> 1) * 2 + (c >> 2)) * 8
            dst[r:r + 8, cols] = v[c]


def _kernel(x_hbm, wqkv_hbm, wo_hbm, w1_hbm, b1_hbm, w2_hbm, b2_hbm, o_hbm,
            spare, sems, x2, w2, w1, b1_raw, b2_raw, out_s, x_in, wqkv_raw, wo_raw, wqkv, w_a, w_b, wo,
            bias1, bias2, xs, x_att, ln1, ln2, qkv_s, qkv_0, o_s):
    n_edge = F // FE

    def qkv_copy(j):
        blk = (_ds((j & 1) * KH, KH), _ds((j >> 1) * D, D))
        return pltpu.make_async_copy(wqkv_hbm.at[blk], wqkv_raw.at[blk], sems.at[j])

    def x_copy(j):
        a, b = ((0, T), (T, 3 * T), (3 * T, S))[j]
        return pltpu.make_async_copy(x_hbm.at[a:b, :], x_in.at[a:b, :], sems.at[6 + j])

    def small_copy(j):
        src, dst = ((wo_hbm, wo_raw), (b1_hbm, b1_raw), (b2_hbm, b2_raw))[j]
        return pltpu.make_async_copy(src, dst, sems.at[9 + j])

    def w1_copy(j):
        cols = _ds(j * FE, FE, 128)
        return pltpu.make_async_copy(w1_hbm.at[:, cols], w1.at[:, cols], sems.at[12 + j])

    def w2_copy(j):
        rows = _ds(j * FE, FE, 128)
        return pltpu.make_async_copy(w2_hbm.at[rows, :], w2.at[rows, :], sems.at[12 + n_edge + j])

    def out_copy(t):
        return pltpu.make_async_copy(out_s.at[t], o_hbm.at[_ds(t * T, T), :], sems.at[12 + 2 * n_edge + t])

    def gate(buf):
        def store(tok):
            if buf.dtype == bf16:
                z = pl.multiple_of(spare[1], 16)
                buf[pl.ds(z, 16), 0:128] = jnp.concatenate([tok, tok], axis=0).astype(bf16)
            else:
                z = pl.multiple_of(spare[0], 8)
                buf[(0,) * (len(buf.shape) - 2) + (pl.ds(z, 8), slice(0, 128))] = tok
        return store

    def put_blocks(buf, c0, r):
        for c in range(r.shape[1] // 128):
            buf[c0 + c, HALO:HALO + T, :] = r[:, c * 128:(c + 1) * 128]

    def first_tile_halo(buf, tile):
        for c in range(2 * NC, 3 * NC):
            v0 = jnp.broadcast_to(buf[c, HALO:HALO + 1, :], (HALO, 128))
            buf[c, 0:HALO, :] = jnp.where(tile == 0, v0, buf[c, 0:HALO, :])

    def attn_rows(buf, r0, pos0):
        def rows(c, w):
            return buf[c, pl.ds(r0 + (HALO - DIL * w), RB), :]
        lg = [None] * W
        for c in range(NC):
            yield True
            q = rows(c, 0)
            for w in range(W):
                t = q * rows(NC + c, w)
                lg[w] = t if c == 0 else lg[w] + t
        t = jnp.concatenate(lg, axis=0)
        lane = jax.lax.broadcasted_iota(i32, t.shape, 1)
        t = t + jnp.take_along_axis(t, lane ^ 1, axis=1)
        t = t + jnp.take_along_axis(t, lane ^ 2, axis=1)
        lg = [t[w * RB:(w + 1) * RB] for w in range(W)]
        if pos0 is not None:
            pos = pos0 + jax.lax.broadcasted_iota(i32, (RB, 128), 0)
            lg = [jnp.where(pos >= DIL * w, lg[w], NEG / SCALE) for w in range(W)]
        m = functools.reduce(jnp.maximum, lg)
        e = [jnp.exp2((t - m) * (SCALE * LOG2E)) for t in lg]
        inv = 1.0 / functools.reduce(jnp.add, e)
        for _ in range(IDLE):
            yield False
        for c in range(NC):
            yield True
            acc = None
            for w in range(W):
                t = e[w] * rows(2 * NC + c, w)
                acc = t if acc is None else acc + t
            o_s[_ds(r0 // 2, RB // 2), c * 128:(c + 1) * 128] = _pack(acc * inv)

    def stream(item, r, nr, cols=slice(None)):
        tile = item & (NT - 1)
        return jnp.where(item < NT, x_in[_ds(tile * T + r, nr), cols].astype(f32), xs[tile, _ds(r, nr), cols])

    def ln1_rows(r, item):
        yield True
        ln1[_ds(r // 2, RB // 2), :] = _pack(_ln(stream(item, r, RB)))

    def ln2_rows(src, r):
        yield True
        ln2[r // 2:(r + RB) // 2, :] = _pack(_ln(src[r:r + RB, :]))

    def ffn_up(cols):
        return _dot(_unpack(ln2[...]), w1[:, cols]) + bias1[0:1, cols]

    def ffn_down(cols, t, acc):
        t = jnp.maximum(t, 0.0)
        return acc + _dot((t * t).astype(bf16), w2[cols, :])

    def store_out(u, y):
        out_s[jnp.maximum(u - NT, 0)] = y.astype(out_s.dtype)

    def share(j, n_iter):
        n = T // RB
        per = -(-n // n_iter)
        return [pl.multiple_of(jnp.minimum(j * per + i, n - 1) * RB, RB) for i in range(per)]

    def start():
        for cp in (x_copy(0), *(qkv_copy(j) for j in range(6)),
                   small_copy(1), small_copy(2), x_copy(1), small_copy(0)):
            cp.start()
        for j in range(n_edge):
            w1_copy(j).start()
            w2_copy(j).start()
        x_copy(2).start()
        spare[0] = HALO + T
        spare[1] = D
        qkv_0[NC:, 0:HALO, :] = jnp.zeros((2 * NC, HALO, 128), f32)

        @pl.loop(0, NT)
        def _(t):
            xs[t, 0:T, :] = jnp.zeros((T, D), f32)
        x_copy(0).wait()
        for r in range(0, T, RB):
            ln2[r // 2:(r + RB) // 2, :] = _pack(_ln(x_in[r:r + RB, :].astype(f32)))
        qkv_copy(0).wait()

        @pl.loop(0, 2)
        def _(j):
            rd = j * (KH // 4)
            _permute_cols(wqkv_raw, j * (KH // 2), 0, [(w_a, rd, 0), (wqkv, rd, 0)], KH // 2)

        @pl.loop(0, 3)
        def _(p):
            for kh, (src, dst) in enumerate(((w_a, w_b), (w_b, w_a))):
                nxt = jnp.minimum(2 * p + kh + 1, 5)

                @pl.when(2 * p + kh < 5)
                def _():
                    qkv_copy(nxt).wait()
                r = _dot(_unpack(ln2[:, kh * KH:(kh + 1) * KH]), _unpack(src[...]))
                for c in range(NC):
                    blk = (p * NC + c, slice(HALO, HALO + T), slice(None))
                    part = r[:, c * 128:(c + 1) * 128]
                    qkv_0[blk] = qkv_0[blk] + part if kh else part
                toks = _vregs(r)
                for s in range(KH // PR):
                    gate(wqkv_raw)(toks[s * 200 // (KH // PR)]())
                    r0, c0 = (1 - kh) * KH + s * PR, (nxt >> 1) * D
                    _permute_cols(wqkv_raw, r0, c0, [(dst, s * PR // 2, 0), (wqkv, r0 // 2, c0)], PR)

        for cp in (small_copy(1), small_copy(2), x_copy(1)):
            cp.wait()
        bias1[...] = jnp.broadcast_to(b1_raw[...].astype(f32).reshape(1, F), (8, F))
        bias2[...] = jnp.broadcast_to(b2_raw[...].astype(f32).reshape(1, D), (8, D))
        for r in range(0, T, RB):
            ln1[r // 2:(r + RB) // 2, :] = _pack(_ln(x_in[T + r:T + r + RB, :].astype(f32)))
        first_tile_halo(qkv_0, 0)
        for c in range(NC, 3 * NC):
            qkv_s[c, 0:HALO, :] = qkv_0[c, T:T + HALO, :]

        @pl.loop(0, 3)
        def _(p):
            r = _dot(_unpack(ln1[...]), _unpack(wqkv[:, _ds(p * D, D)]))
            put_blocks(qkv_s, p * NC, r)
            pieces = share(p, 3)
            ga = _steps(*(attn_rows(qkv_0, r0, r0) for r0 in pieces))
            _paced(ga, len(pieces) * SLOTS, _vregs(r)[:210], gate(qkv_0))
            _drain(ga)
        small_copy(0).wait()

        @pl.loop(0, D // 256)
        def _(c):
            _permute_rows(wo_raw, wo, c * 256, 256)

    def steady(u):
        cur = (u + 1) & (NT - 1)
        for c in range(NC, 3 * NC):
            qkv_s[c, 0:HALO, :] = qkv_s[c, T:T + HALO, :]
        x2[0:T, :] = stream(u, 0, T) + _dot(_unpack(o_s[...]), _unpack(wo[...]))
        toks = []
        a = _unpack(ln1[...])
        for p in range(3):
            r = _dot(a, _unpack(wqkv[:, p * D:(p + 1) * D]))
            put_blocks(qkv_s, p * NC, r)
            toks += _vregs(r)
        g2 = _steps(*(ln2_rows(x2, r) for r in range(0, T, RB)))
        _paced(g2, T // RB, toks[:384], gate(x2))
        _drain(g2)
        first_tile_halo(qkv_s, cur)

        def quota(n, h0, h1, h):
            return (h - h0 + 1) * n // (h1 - h0) - (h - h0) * n // (h1 - h0) if h0 <= h < h1 else 0
        acc = x2[0:T, :] + bias2[0:1, :]
        ga = _steps(*(attn_rows(qkv_s, r0, cur * T + r0 if r0 < HALO else None) for r0 in range(0, T, RB)))
        g1 = _steps(*(ln1_rows(r, u + 2) for r in range(0, T, RB)))
        for j in range(F // FC):
            cols = pl.ds(j * FC, FC)
            n = quota((T // RB) * SLOTS, 0, 6, j)
            t = ffn_up(cols)
            _paced(g1, quota(T // RB, 12, 13, 2 * j), _vregs(t), gate(xs))
            _paced(ga, n // 3, _vregs(t), gate(qkv_s))
            acc = ffn_down(cols, t, acc)
            _paced(g1, quota(T // RB, 12, 13, 2 * j + 1), _vregs(acc), gate(xs))
            _paced(ga, n - n // 3, _vregs(acc), gate(qkv_s))
        _drain(ga)
        _drain(g1)
        xs[u & (NT - 1), 0:T, :] = acc
        store_out(u, acc)

    def edge(u):
        @pl.loop(0, 2)
        def _(j):
            cols = _ds(j * (D // 2), D // 2)
            x = stream(u, 0, T, cols) + _dot(_unpack(o_s[...]), _unpack(wo[:, cols]))
            x_att[:, cols] = x
            x2[0:T, cols] = x + bias2[0:1, cols]
        _drain(_steps(*(ln2_rows(x_att, r) for r in range(0, T, RB))))

        @pl.loop(0, n_edge)
        def _(j):
            @pl.when(u == 0)
            def _():
                w1_copy(j).wait()
                w2_copy(j).wait()
            cols = _ds(j * FE, FE, 128)
            t = ffn_up(cols)
            pieces = share(j, n_edge)
            pos = ((u + 1) & (NT - 1)) * T
            ga = _steps(*(attn_rows(qkv_s, r0, pos + r0) for r0 in pieces))
            n = len(pieces) * SLOTS
            _paced(ga, n * 2 // 3, _vregs(t), gate(qkv_s))
            acc = ffn_down(cols, t, x2[0:T, :])
            x2[0:T, :] = acc
            _paced(ga, n - n * 2 // 3, _vregs(acc)[:100], gate(qkv_s))
            _drain(ga)
            g1 = _steps(*(ln1_rows(r, u + 2) for r in pieces))
            _paced(g1, len(pieces), _vregs(acc)[100:220], gate(xs))
            _drain(g1)

        @pl.when(u == 0)
        def _():
            xs[0, 0:T, :] = x2[0:T, :]
            x_copy(2).wait()

        @pl.when(u != 0)
        def _():
            store_out(u, x2[0:T, :])

    start()

    @pl.loop(0, NI)
    def _(u):
        is_edge = jnp.logical_or(u == 0, u == NI - 1)
        pl.when(jnp.logical_not(is_edge))(lambda: steady(u))
        pl.when(is_edge)(lambda: edge(u))
        pl.when(u >= NT)(lambda: out_copy(u - NT).start())

    for t in range(NT):
        out_copy(t).wait()


@jax.jit
def pallas_interleave_layers__sliding_local_dilated__dense_activation_squared_relu__prompt_kernel(
    A_x: jax.Array,
    A_wqkv: jax.Array,
    A_wo: jax.Array,
    B_x: jax.Array,
    B_w1: jax.Array,
    B_b1: jax.Array,
    B_w2: jax.Array,
    B_b2: jax.Array,
):
    del B_x
    vm = pltpu.VMEM
    hbm = pl.BlockSpec(memory_space=pl.ANY)
    out = pl.pallas_call(
        _kernel,
        in_specs=[hbm] * 7,
        out_specs=hbm,
        out_shape=jax.ShapeDtypeStruct((S, D), A_x.dtype),
        scratch_shapes=[
            pltpu.SMEM((2,), i32),
            pltpu.SemaphoreType.DMA((12 + 2 * (F // FE) + NT,)),
            vm((T + HALO + 8, D), f32),
            vm((F, D), bf16), vm((D, F), bf16),
            vm((F,), bf16), vm((D,), bf16),
            vm((NT, T, D), A_x.dtype), vm((S, D), A_x.dtype),
            vm((D + 16, 3 * D), bf16), vm((D, D), bf16),
            vm((KH, 3 * D), i32),
            vm((KH // 2, D), i32), vm((KH // 2, D), i32),
            vm((KH, D), i32),
            vm((8, F), f32), vm((8, D), f32),
            vm((NT, T + HALO + 8, D), f32), vm((T, D), f32),
            vm((T // 2, D), i32), vm((T // 2, D), i32),
            vm((3 * NC, HALO + T + 8, 128), f32),
            vm((3 * NC, HALO + T + 8, 128), f32),
            vm((T // 2, D), i32),
        ],
        compiler_params=pltpu.CompilerParams(vmem_limit_bytes=110 * 2**20),
    )(A_x.reshape(S, D), A_wqkv, A_wo, B_w1, B_b1, B_w2, B_b2)
    return out.reshape(A_x.shape)
```
